```python
import jax
import jax.numpy as jnp

def _softmax(x, axis=-1):
    return jax.nn.softmax(x, axis=axis)

def _gelu(x):
    return jax.nn.gelu(x, approximate=True)

def _silu(x):
    return jax.nn.silu(x)

def _sigmoid(x):
    return jax.nn.sigmoid(x)

def _layernorm(x, axis=-1, eps=1e-05):
    m = jnp.mean(x, axis=axis, keepdims=True)
    v = jnp.var(x, axis=axis, keepdims=True)
    return (x - m) / jnp.sqrt(v + eps)

def _scatter_add(tgt, idx, src, axis=0):
    return tgt.at[idx].add(src)

def _segment_sum(src, seg, n):
    return jax.ops.segment_sum(src, seg, n)

class _Rng:

    def __init__(self, key):
        self._k = key

    def _next(self):
        self._k, sub = jax.random.split(self._k)
        return sub

    def normal(self, shape):
        return jax.random.normal(self._next(), shape, dtype=jnp.bfloat16)

    def randint(self, lo, hi, shape):
        return jax.random.randint(self._next(), shape, lo, hi, dtype=jnp.int32)

    def uniform(self, shape, lo=0.0, hi=1.0):
        return jax.random.uniform(self._next(), shape, jnp.bfloat16, lo, hi)

    def permutation(self, n):
        return jax.random.permutation(self._next(), n)
kernel_name = 'adaLN_cond__sliding_block_cached__dense_activation_mish__decode'

def setup_inputs():
    _rng = _Rng(jax.random.key(int.from_bytes(__import__("os").urandom(4), "little")))
    _w = lambda a: (lambda t: t.astype(jnp.bfloat16) if jnp.issubdtype(t.dtype, jnp.floating) else t)(jnp.asarray(a))

    def _A_setup():
        B, Sq, D = (1, 1, 640)
        Hq, Hkv, Sk, Dh = (32, 32, 32768, 192)
        assert Hq % Hkv == 0, (Hq, Hkv)
        return {'x': _w((lambda *s: _rng.normal(s) * 0.05)(B, Sq, D)), 'k_cache': _w((lambda *s: _rng.normal(s) * 0.05)(B, Hkv, Sk, Dh)), 'v_cache': _w((lambda *s: _rng.normal(s) * 0.05)(B, Hkv, Sk, Dh)), 'wq': _w((lambda *s: _rng.normal(s) * 0.05)(D, Hq * Dh) * D ** (-0.5)), 'wo': _w((lambda *s: _rng.normal(s) * 0.05)(Hq * Dh, D) * (Hq * Dh) ** (-0.5))}
    _A_in = _A_setup()

    def _B_setup():
        B, S, D, F = (1, 1, 640, 1536)
        return {'x': _w((lambda *s: _rng.normal(s) * 0.05)(B, S, D)), 'w1': _w((lambda *s: _rng.normal(s) * 0.05)(D, F) * D ** (-0.5)), 'b1': _w((lambda *s: _rng.normal(s) * 0.05)(F)), 'w2': _w((lambda *s: _rng.normal(s) * 0.05)(F, D) * F ** (-0.5))}
    _B_in = _B_setup()
    return {'A_x': _A_in['x'], 'A_k_cache': _A_in['k_cache'], 'A_v_cache': _A_in['v_cache'], 'A_wq': _A_in['wq'], 'A_wo': _A_in['wo'], 'B_x': _B_in['x'], 'B_w1': _B_in['w1'], 'B_b1': _B_in['b1'], 'B_w2': _B_in['w2'], 'c': _w((lambda *s: _rng.normal(s) * 0.05)(1, 640)), 'w_mod': _w((lambda *s: _rng.normal(s) * 0.05)(640, 6 * 640) * 640 ** (-0.5))}

def reference(A_x, A_k_cache, A_v_cache, A_wq, A_wo, B_x, B_w1, B_b1, B_w2, c, w_mod):

    def _A_ref(x, k_cache, v_cache, wq, wo):
        B, Sq, D = x.shape
        Hq, Dh = (32, 192)
        Hkv, Sk = (k_cache.shape[1], k_cache.shape[2])
        W = min(4096, max(256, Sk // 4))
        rep = Hq // Hkv
        q = (lambda x, *d: x.transpose(*d))((x @ wq).reshape(B, Sq, Hq, Dh), 0, 2, 1, 3)
        k = jnp.repeat(k_cache[:, :, Sk - W:, :], rep, axis=1)
        v = jnp.repeat(v_cache[:, :, Sk - W:, :], rep, axis=1)
        scores = jnp.einsum('bhqd,bhkd->bhqk', q, k) * Dh ** (-0.5)
        p = _softmax(scores, axis=-1)
        o = jnp.einsum('bhqk,bhkd->bhqd', p, v)
        return (lambda x, *d: x.transpose(*d))(o, 0, 2, 1, 3).reshape(B, Sq, Hq * Dh) @ wo

    def _B_ref(x, w1, b1, w2):
        h = jnp.einsum('bsd,df->bsf', x, w1) + b1
        sp = jnp.log1p(jnp.exp(-jnp.abs(h))) + jnp.where(h > 0, h, jnp.zeros_like(h))
        act = h * jnp.tanh(sp)
        return jnp.einsum('bsf,fd->bsd', act, w2)
    x = A_x
    mod = (_silu(c) @ w_mod).reshape(c.shape[0], 6, 1, -1)
    sa, ca, ga, sb, cb, gb = (mod[:, 0].copy(), mod[:, 1].copy(), mod[:, 2].copy(), mod[:, 3].copy(), mod[:, 4].copy(), mod[:, 5].copy())
    h = _layernorm(x, axis=-1) * (1 + ca) + sa
    x = x + ga * _A_ref(h, A_k_cache, A_v_cache, A_wq, A_wo)
    h = _layernorm(x, axis=-1) * (1 + cb) + sb
    x = x + gb * _B_ref(h, B_w1, B_b1, B_w2)
    return x
```

```python
import functools

import jax
import jax.numpy as jnp
from jax import lax
import jax.experimental.pallas as pl
import jax.experimental.pallas.tpu as pltpu

D = 640
H = 32
DH = 192
F = 1536
PAIR = 2 * DH
NPAIR = H // 2
LANE = 128
SUB = 8
PIECE = 4
STRIPE = 64
F32 = jnp.float32
BF16 = jnp.bfloat16

DEFAULT = dict(
    cycle=(0, 1, 1, 1, 1, 1),
    kvcycle=((1, 0), (1, 1), (1, 1), (1, 1), (1, 1), (1, 1)),
    run=24,
    nslot=3,
    look_a=200,
    pace=40,
    w1_late=0,
    look_v14=384,
    look_v=96,
    look_m=96,
    pace_t=20,
    w2_parts=(((0, 256), (384, 256), (768, 256), (1152, 256)), ((256, 128), (640, 128)), ((1024, 128),), ((1408, 128),)),
    w2_rows=(8, 8, 8, 8),
    w2_cycle=(0, 1, 1, 1, 1, 1),
    w2_lead=24,
    pace_v=16,
    pace_14=16,
    shift=0,
    wshift=0,
    bounds=False,
    compute=True,
    groups=(("wmod", "w1"), ("wq", "wo")),
    fence=True,
    last_cols=True,
    marks=False,
)


def _layernorm(x, eps=1e-5):
    m = jnp.mean(x, axis=-1, keepdims=True)
    d = x - m
    v = jnp.mean(d * d, axis=-1, keepdims=True)
    return d / jnp.sqrt(v + eps)


def _mish(u):
    softplus = jnp.log1p(jnp.exp(-jnp.abs(u))) + jnp.where(u > 0, u, 0.0)
    return u * jnp.tanh(softplus)


def _dot(a, b):
    return jnp.dot(a, b, preferred_element_type=F32)


def _dot_nt(a, b):
    return lax.dot_general(a, b, (((1,), (1,)), ((), ())), preferred_element_type=F32)


def _piece(src, dst, sem, i):
    width = src.shape[1] // LANE
    out, t, end = [], i * PIECE, (i + 1) * PIECE
    while t < end:
        r, c = divmod(t, width)
        n = min(end - t, width - c)
        idx = (pl.ds(r * SUB, SUB), pl.ds(c * LANE, n * LANE))
        out.append(functools.partial(pltpu.make_async_copy, src.at[idx], dst.at[idx], sem))
        t += n
    return out


def _npieces(ref):
    return ref.shape[0] * ref.shape[1] // (PIECE * SUB * LANE)


class _Stream:
    def __init__(self, parts, fence=None):
        self.items = [it for part in parts for it in part]
        self.ends = []
        n = 0
        for part in parts:
            n += len(part)
            self.ends.append(n)
        self.fence = fence
        self.pos = 0

    def upto(self, n):
        n = min(n, len(self.items))
        while self.pos < n:
            if self.fence is not None and self.pos in self.ends:
                self.fence()
            prio, copies = self.items[self.pos]
            for cp in copies:
                cp().start(priority=prio)
            self.pos += 1

    def more(self, k):
        self.upto(self.pos + k)

    def past(self, part, look):
        self.upto(self.ends[part] + look)

    def rest(self):
        self.upto(len(self.items))


def _wait_all(buf, sem):
    pltpu.make_async_copy(buf, buf, sem).wait()


def _kernel(x_hbm, k_hbm, v_hbm, wq_hbm, wo_hbm, w1_hbm, b1_hbm, w2_hbm, c_hbm, wmod_hbm, o_ref,
            x_v, c_v, b1_v, wmod_v, wq_v, wo_v, w1_v, w2_v, ring, p_s, att_s, mod_s,
            sem_w, sem_kv, sem_last, sem_w2, sem_fence, *, window, cfg):
    sk = k_hbm.shape[1]
    wide = PIECE * LANE
    ncol = window // wide
    nslot = cfg["nslot"]
    compute = cfg["compute"]

    def mark(name):
        if cfg["marks"]:
            with jax.named_scope(name):
                pl.semaphore_signal(sem_fence, 1)
                pl.semaphore_wait(sem_fence, 1)

    def aligned(i):
        return i if isinstance(i, int) else pl.multiple_of(i, LANE)

    def rolled(items, k):
        zero = [it for it in items if it[0] == 0]
        zero = iter(zero[len(zero) - k:] + zero[:len(zero) - k])
        return [next(zero) if it[0] == 0 else it for it in items]

    def queued(pieces):
        cyc = cfg["cycle"]
        return rolled([(cyc[i % len(cyc)], cps) for i, cps in enumerate(pieces)], cfg["wshift"])

    def kv_items(src, p, slot, run=cfg["run"], sems=None):
        out, j = [], 0
        cyc = cfg["kvcycle"]
        src = src.at[pl.ds(aligned(p * PAIR), PAIR), pl.ds(sk - window, window)]
        dst = ring.at[slot]
        sem = sem_kv.at[slot]
        for r0 in range(0, PAIR // SUB, run):
            for c in reversed(range(ncol)):
                r = r0
                while r < r0 + run:
                    n, prio = cyc[j % len(cyc)]
                    j += 1
                    idx = (pl.ds(r * SUB, n * SUB), pl.ds(c * wide, wide))
                    out.append((prio, [functools.partial(
                        pltpu.make_async_copy, src.at[idx], dst.at[idx], sem if sems is None else sems.at[c])]))
                    r += n
                assert r == r0 + run
        return out if sems is not None else rolled(out, cfg["shift"])

    def fence():
        pl.semaphore_signal(sem_fence, 1)
        pl.semaphore_wait(sem_fence, 1)

    if not cfg["fence"]:
        fence = None

    s_c, s_x, s_b1, s_wmod, s_wq, s_wo, s_w1, s_w1_late = range(8)
    small = [functools.partial(pltpu.make_async_copy, s, d, sem_w.at[i])
             for i, s, d in ((s_c, c_hbm, c_v), (s_x, x_hbm, x_v), (s_b1, b1_hbm, b1_v))]
    mats = dict(wmod=(wmod_hbm, wmod_v, s_wmod), wq=(wq_hbm, wq_v, s_wq), wo=(wo_hbm, wo_v, s_wo), w1=(w1_hbm, w1_v, s_w1))
    nb1 = F // wide
    early1 = nb1 - cfg["w1_late"]

    def walk(names):
        out = []
        for c in reversed(range(STRIPE)):
            for nm in names:
                src, dst, s = mats[nm]
                for i in range(c, _npieces(src), STRIPE):
                    if nm == "w1" and i % nb1 >= early1:
                        continue
                    out.append(_piece(src, dst, sem_w.at[s], i))
        return out

    def sweep(nm, period, i):
        src, dst, s = mats[nm]
        rows = period * PIECE * LANE // src.shape[1] * SUB
        r0 = i * rows if isinstance(i, int) else pl.multiple_of(i * rows, SUB)
        n = src.shape[0] - (STRIPE // period - 1) * rows
        src, dst = src.at[pl.ds(r0, n)], dst.at[pl.ds(r0, n)]
        return queued([_piece(src, dst, sem_w.at[s], r + c)
                       for c in reversed(range(period)) for r in range(0, _npieces(mats[nm][0]), STRIPE)])

    def edge(nm, first):
        src, dst, s = mats[nm]
        return queued([_piece(src, dst, sem_w.at[s], r + c)
                       for c in reversed(range(first, STRIPE)) for r in range(0, _npieces(src), STRIPE)])

    head = _Stream([queued(walk(("wmod", "w1"))), edge("wo", 60)], fence)
    head.upto(6)
    for cp in small:
        cp().start()
    head.rest()
    mark("m_A1")

    @pl.loop(0, 12)
    def _(i):
        _Stream([sweep("wo", 5, 11 - i)]).rest()

    mark("m_wo")
    _Stream([edge("wq", 60)]).rest()
    for cp in small:
        cp().wait()
    _wait_all(wmod_v, sem_w.at[s_wmod])
    cf = c_v[...].astype(F32)
    silu_c = jnp.broadcast_to(cf * jax.nn.sigmoid(cf), (8, D)).astype(BF16)

    @pl.loop(0, 5)
    def _(i):
        stream = _Stream([sweep("wq", 12, 4 - i)])
        n = 6 * D // 5
        for j in range(2):
            cols = pl.ds(aligned(i * n + j * n // 2), n // 2)
            stream.more(60)
            mod_s[:, cols] = _dot(silu_c, wmod_v[:, cols]) if compute else jnp.zeros((8, n // 2), F32)
        stream.rest()

    mark("m_wq")

    def mod(i):
        return mod_s[:, i * D:(i + 1) * D]

    x0 = jnp.broadcast_to(x_v[...].astype(F32), (8, D))
    h = (_layernorm(x0) * (1.0 + mod(1)) + mod(0)).astype(BF16)

    @pl.loop(0, 2)
    def _(p):
        _Stream([kv_items(k_hbm, p, p)]).rest()

    _wait_all(wq_v, sem_w.at[s_wq])
    _wait_all(wo_v, sem_w.at[s_wo])
    if early1:
        _wait_all(w1_v.at[:, pl.ds(0, early1 * wide)], sem_w.at[s_w1])
    att_s[...] = jnp.zeros(att_s.shape, F32)
    row = lax.broadcasted_iota(jnp.int32, (8, PAIR), 0)
    col = lax.broadcasted_iota(jnp.int32, (8, PAIR), 1)
    own = jnp.logical_or(jnp.logical_and(row == 0, col < DH), jnp.logical_and(row == 1, col >= DH))

    def scores(p, slot, stream):
        step = len(stream.items) // (ncol + 2)
        _wait_all(ring.at[slot], sem_kv.at[slot])
        if compute:
            q = jnp.where(own, _dot(h, wq_v[:, pl.ds(aligned(p * PAIR), PAIR)]), 0.0).astype(BF16)
            stream.more(step)
            s = []
            for c in range(ncol):
                s.append(_dot(q, ring[slot, :, c * wide:(c + 1) * wide]) * DH ** -0.5)
                stream.more(step)
            s = jnp.concatenate(s, axis=1)
            e = jnp.exp(s - jnp.max(s, axis=-1, keepdims=True))
            p_s[p] = e / jnp.sum(e, axis=-1, keepdims=True)
        stream.rest()

    def project(p, acc):
        return _dot(jnp.where(own, acc, 0.0).astype(BF16), wo_v[pl.ds(aligned(p * PAIR), PAIR), :])

    def pv(p, slot, c):
        cols = pl.ds(c * wide, wide)
        return _dot_nt(p_s[p, :, cols].astype(BF16), ring[slot, :, cols])

    def values(p, slot, stream, step):
        _wait_all(ring.at[slot], sem_kv.at[slot])
        if compute:
            acc = jnp.zeros((8, PAIR), F32)
            for c in range(ncol):
                acc += pv(p, slot, c)
                stream.more(step)
            att_s[...] += project(p, acc)

    def k_body(p, carry):
        scores(p, p % nslot, _Stream([kv_items(k_hbm, p + 2, (p + 2) % nslot)]))
        return carry

    mark("m_k01")
    lax.fori_loop(0, NPAIR - 2, k_body, 0)
    mark("m_K")

    @pl.loop(NPAIR - 2, NPAIR)
    def _(p):
        scores(p, p % nslot, _Stream([kv_items(v_hbm, p + 2 - NPAIR, (p + 2) % nslot)]))

    def v_body(p, carry):
        stream = _Stream([kv_items(v_hbm, p + 2, (NPAIR + p + 2) % nslot)])
        values(p, (NPAIR + p) % nslot, stream, len(stream.items) // (ncol + 2))
        stream.rest()
        return carry

    mark("m_K2")
    lax.fori_loop(0, NPAIR - 3, v_body, 0)
    mark("m_V")

    parts = cfg["w2_parts"]
    n2 = cfg["w2_rows"]
    flat, sizes = [], []
    for i, part in enumerate(parts):
        m = n2[i]
        cps = [[functools.partial(pltpu.make_async_copy, w2_hbm.at[pl.ds(r0 + r, m)], w2_v.at[pl.ds(r0 + r, m)], sem_w2.at[i])]
               for r in range(0, part[0][1], m) for r0, n in part if r < n]
        flat += cps
        sizes.append(len(cps))
    cyc = cfg["w2_cycle"]
    flat = [(cyc[i % len(cyc)], cps) for i, cps in enumerate(flat)]
    ones = [it for it in flat if it[0] == 1]
    zeros = [it for it in flat if it[0] == 0]
    k = cfg["w2_lead"]
    flat = ones[:k]
    rest = ones[k:]
    for i, it in enumerate(zeros):
        flat += [it] + rest[i * len(rest) // len(zeros):(i + 1) * len(rest) // len(zeros)]
    cut = [flat]
    last = NPAIR - 1
    slot = (NPAIR + last) % nslot
    if cfg["last_cols"]:
        v15 = kv_items(v_hbm, last, slot, PAIR // SUB, sem_last)
        per = len(v15) // ncol
        v15 = [v15[i * per:(i + 1) * per] for i in range(ncol)]
    else:
        v15 = [kv_items(v_hbm, last, slot)]
    nv = len(v15)
    tail = _Stream(v15 + cut, fence)
    nitem = tail.ends[nv - 1]
    values(last - 2, (slot - 2) % nslot, tail, nitem // (3 * ncol))
    mark("m_v13")
    tail.upto(min(nitem // 2, cfg["look_v14"]))
    values(last - 1, (slot - 1) % nslot, tail, cfg["pace_14"])
    mark("m_v14")
    acc = jnp.zeros((8, PAIR), F32)
    if cfg["last_cols"]:
        for i, c in enumerate(reversed(range(ncol))):
            tail.more(cfg["pace_v"])
            tail.past(i, cfg["look_v"] if i < ncol - 1 else cfg["look_m"])
            _wait_all(ring.at[slot, :, pl.ds(c * wide, wide)], sem_last.at[c])
            mark(f"m_c{c}")
            if compute:
                acc += pv(last, slot, c)
    else:
        tail.past(0, cfg["look_v"])
        _wait_all(ring.at[slot], sem_kv.at[slot])
        for c in range(ncol):
            if compute:
                acc += pv(last, slot, c)
            tail.more(cfg["pace_t"])
    tail.more(cfg["pace_t"])
    att = att_s[...] + project(last, acc) if compute else acc[:, :1]
    tail.more(cfg["pace_t"])

    att = jnp.broadcast_to(jnp.sum(att, axis=0, keepdims=True), (8, D))
    x1 = x0 + mod(2) * att
    h2 = (_layernorm(x1) * (1.0 + mod(4)) + mod(3)).astype(BF16)
    tail.more(cfg["pace_t"])
    mark("m_h2")
    b1 = b1_v[...].astype(F32)
    acts = []
    for i in range(nb1):
        bias = jnp.concatenate(
            [jnp.broadcast_to(b1[t:t + 1, :], (8, LANE)) for t in range(i * PIECE, (i + 1) * PIECE)], axis=1)
        if compute:
            acts.append(_mish(_dot(h2, w1_v[:, i * wide:(i + 1) * wide]) + bias).astype(BF16))
        tail.more(cfg["pace_t"])
    tail.rest()
    act = jnp.concatenate(acts, axis=1) if compute else None
    mark("m_act")
    y = jnp.zeros((8, D), F32)
    for i, part in enumerate(parts):
        _wait_all(w2_v.at[pl.ds(0, sum(n for _, n in part))], sem_w2.at[i])
        mark(f"m_w{i}")
        if compute:
            for r0, n in part:
                y += _dot(act[:, r0:r0 + n], w2_v[r0:r0 + n, :])
    o_ref[...] = (x1 + mod(5) * y)[0:1].astype(o_ref.dtype)


def make(**kw):
    cfg = dict(DEFAULT, **kw)

    def fn(A_x, A_k_cache, A_v_cache, A_wq, A_wo, B_x, B_w1, B_b1, B_w2, c, w_mod):
        del B_x
        sk = A_k_cache.shape[2]
        window = min(4096, max(256, sk // 4))
        kt = jnp.swapaxes(A_k_cache, 2, 3).reshape(H * DH, sk)
        vt = jnp.swapaxes(A_v_cache, 2, 3).reshape(H * DH, sk)
        hbm = pl.BlockSpec(memory_space=pltpu.HBM)
        out = pl.pallas_call(
            functools.partial(_kernel, window=window, cfg=cfg),
            out_shape=jax.ShapeDtypeStruct((1, D), A_x.dtype),
            in_specs=[hbm] * 10,
            out_specs=pl.BlockSpec(memory_space=pltpu.VMEM),
            scratch_shapes=[
                pltpu.VMEM((1, D), BF16),
                pltpu.VMEM((1, D), BF16),
                pltpu.VMEM((F // LANE, LANE), BF16),
                pltpu.VMEM((D, 6 * D), BF16),
                pltpu.VMEM((D, H * DH), BF16),
                pltpu.VMEM((H * DH, D), BF16),
                pltpu.VMEM((D, F), BF16),
                pltpu.VMEM((F, D), BF16),
                pltpu.VMEM((cfg["nslot"], PAIR, window), BF16),
                pltpu.VMEM((NPAIR, 8, window), F32),
                pltpu.VMEM((8, D), F32),
                pltpu.VMEM((8, 6 * D), F32),
                pltpu.SemaphoreType.DMA((8,)),
                pltpu.SemaphoreType.DMA((cfg["nslot"],)),
                pltpu.SemaphoreType.DMA((window // (PIECE * LANE),)),
                pltpu.SemaphoreType.DMA((len(cfg["w2_parts"]),)),
                pltpu.SemaphoreType.REGULAR,
            ],
            compiler_params=pltpu.CompilerParams(
                vmem_limit_bytes=64 * 2**20,
                disable_semaphore_checks=True,
                disable_bounds_checks=not cfg["bounds"],
            ),
            name="adaln_attn_mlp_decode",
        )(A_x.reshape(1, D), kt, vt, A_wq, A_wo, B_w1, B_b1.reshape(F // LANE, LANE), B_w2, c, w_mod)
        return out.reshape(A_x.shape)

    return fn


@jax.jit
def pallas_adaLN_cond__sliding_block_cached__dense_activation_mish__decode_kernel(
    A_x, A_k_cache, A_v_cache, A_wq, A_wo, B_x, B_w1, B_b1, B_w2, c, w_mod):
    return make()(A_x, A_k_cache, A_v_cache, A_wq, A_wo, B_x, B_w1, B_b1, B_w2, c, w_mod)
```

```python
import functools

import jax
import jax.numpy as jnp
from jax import lax
import jax.experimental.pallas as pl
import jax.experimental.pallas.tpu as pltpu

D = 640
H = 32
DH = 192
F = 1536
PAIR = 2 * DH
NPAIR = H // 2
LANE = 128
SUB = 8
PIECE = 4
WIDE = PIECE * LANE
STRIPE = 64
F32 = jnp.float32
BF16 = jnp.bfloat16

NSLOT = 3
KV_COLS = (5, 6, 7, 4, 3, 0, 1, 2)
KV_CYCLE = ((0, 1), (1, 2), (1, 1), (1, 2))
W_CYCLE = (0, 1, 1, 1, 1, 1)
KV_LAG, W_LAG, W2_LAG = 8, 5, 4
W2_MXU = (((0, 256), (384, 256), (768, 256), (1152, 128)), ((256, 128), (640, 128), (1024, 128)))
W2_VPU = ((1280, 128), (1408, 64), (1472, 48), (1520, 16))
V_PACE, V_LOOK = 11, 64
MLP_PACE, MLP_LOOK = 20, 96


def _layernorm(x, eps=1e-5):
    m = jnp.mean(x, axis=-1, keepdims=True)
    d = x - m
    v = jnp.mean(d * d, axis=-1, keepdims=True)
    return d / jnp.sqrt(v + eps)


def _mish(u):
    softplus = jnp.log1p(jnp.exp(-jnp.abs(u))) + jnp.where(u > 0, u, 0.0)
    return u * jnp.tanh(softplus)


def _dot(a, b):
    return jnp.dot(a, b, preferred_element_type=F32)


def _aligned(i, n):
    return i if isinstance(i, int) else pl.multiple_of(i, n)


def _copy(src, dst, sem, idx, queue):
    pltpu.make_async_copy(src.at[idx], dst.at[idx], sem).start(priority=queue)


def _wait_all(buf, sem):
    pltpu.make_async_copy(buf, buf, sem).wait()


def _piece(src, dst, sem, i):
    width = src.shape[1] // LANE
    starts, t, end = [], i * PIECE, (i + 1) * PIECE
    while t < end:
        r, c = divmod(t, width)
        n = min(end - t, width - c)
        starts.append(functools.partial(_copy, src, dst, sem, (pl.ds(r * SUB, SUB), pl.ds(c * LANE, n * LANE))))
        t += n
    return starts


def _queued(pieces):
    return [(W_CYCLE[i % len(W_CYCLE)], starts) for i, starts in enumerate(pieces)]


def _walk(mats, cols):
    return _queued([_piece(*m, i) for c in cols for m in mats
                    for i in range(c, m[0].size // (SUB * WIDE), STRIPE)])


def _sweep(mat, period, i):
    src, dst, sem = mat
    rows = period * WIDE // src.shape[1] * SUB
    view = pl.ds(_aligned(i * rows, SUB), src.shape[0] - (STRIPE // period - 1) * rows)
    return _queued([_piece(src.at[view], dst.at[view], sem, r + c) for c in reversed(range(period))
                    for r in range(0, src.size // (SUB * WIDE), STRIPE)])


def _held(seq, lag):
    zero = [x for x in seq if x[0] == 0]
    return zero[len(zero) - lag:]


def _lagged(seq, lag, held=(), valid=None):
    if valid is not None:
        held = [(0, [lambda q, s=s: pl.when(valid)(lambda: s(q)) for s in starts]) for _, starts in held]
    zero = [x for x in seq if x[0] == 0]
    zero = iter([None] * (lag - len(held)) + list(held) + zero[:len(zero) - lag])
    return [x for x in (next(zero) if x[0] == 0 else x for x in seq) if x is not None]


class _Stream:
    def __init__(self, seq):
        self.seq = seq
        self.pos = 0

    def upto(self, n):
        while self.pos < min(n, len(self.seq)):
            queue, starts = self.seq[self.pos]
            for start in starts:
                start(queue)
            self.pos += 1

    def more(self, n):
        self.upto(self.pos + n)

    def rest(self):
        self.upto(len(self.seq))


def _kernel(x_hbm, k_hbm, v_hbm, wq_hbm, wo_hbm, w1_hbm, b1_hbm, w2_hbm, c_hbm, wmod_hbm, o_ref,
            x_v, c_v, b1_v, wmod_v, wq_v, wo_v, w1_v, w2_v, ring, p_s, att_s, mod_s, act_s,
            sem_w, sem_kv, sem_last, sem_w2):
    window = ring.shape[2]
    ncol = len(KV_COLS)
    assert window == ncol * WIDE
    small = [pltpu.make_async_copy(s, d, sem_w.at[i])
             for i, (s, d) in enumerate(((c_hbm, c_v), (x_hbm, x_v), (b1_hbm, b1_v)))]
    wmod, wq, wo, w1 = [(s, d, sem_w.at[len(small) + i]) for i, (s, d) in enumerate(
        ((wmod_hbm, wmod_v), (wq_hbm, wq_v), (wo_hbm, wo_v), (w1_hbm, w1_v)))]

    def pair(src, base, p, run=DH // SUB, sems=None):
        slot = (base + p) % NSLOT
        src = src.at[pl.ds(_aligned(p * PAIR, LANE), PAIR), pl.ds(src.shape[1] - window, window)]
        dst, sem = ring.at[slot], sem_kv.at[slot]
        seq = []
        for r0 in range(0, PAIR // SUB, run):
            for c in KV_COLS:
                r = r0
                while r < r0 + run:
                    queue, n = KV_CYCLE[len(seq) % len(KV_CYCLE)]
                    idx = (pl.ds(r * SUB, n * SUB), pl.ds(c * WIDE, WIDE))
                    seq.append((queue, [functools.partial(
                        _copy, src, dst, sem if sems is None else sems.at[c], idx)]))
                    r += n
                assert r == r0 + run
        return seq

    def pair_stream(src, base, p, maybe_first=False):
        held = _held(pair(src, base, jnp.maximum(p - 1, 0)), KV_LAG)
        return _Stream(_lagged(pair(src, base, p), KV_LAG, held, p > 0 if maybe_first else None))

    def sweep_stream(mat, period, i):
        last = STRIPE // period - 1
        held = _held(_sweep(mat, period, jnp.minimum(last - i + 1, last)), W_LAG)
        return _Stream(_lagged(_sweep(mat, period, last - i), W_LAG, held, i > 0))

    odd_cols = range(STRIPE - 1, 59, -1)
    seq = _walk((wmod, w1), range(STRIPE - 1, -1, -1)) + _walk((wo,), odd_cols)
    stream = _Stream(_lagged(seq, W_LAG) + _held(seq, W_LAG))
    stream.more(len(W_CYCLE))
    for cp in small:
        cp.start()
    stream.rest()

    @pl.loop(0, 12)
    def _(i):
        sweep_stream(wo, 5, i).rest()

    seq = _walk((wq,), odd_cols)
    _Stream(_lagged(seq, W_LAG, _held(_sweep(wo, 5, 0), W_LAG)) + _held(seq, W_LAG)).rest()
    for cp in small:
        cp.wait()
    _wait_all(*wmod[1:])
    cf = c_v[...].astype(F32)
    silu_c = jnp.broadcast_to(cf * jax.nn.sigmoid(cf), (8, D)).astype(BF16)

    @pl.loop(0, 5)
    def _(i):
        stream = sweep_stream(wq, 12, i)
        n = 6 * D // 10
        for j in range(2):
            stream.more(len(stream.seq) // 3)
            cols = pl.ds(_aligned((2 * i + j) * n, LANE), n)
            mod_s[:, cols] = _dot(silu_c, wmod_v[:, cols])
        stream.rest()

    def mod(i):
        return mod_s[:, i * D:(i + 1) * D]

    x0 = jnp.broadcast_to(x_v[...].astype(F32), (8, D))
    h = (_layernorm(x0) * (1.0 + mod(1)) + mod(0)).astype(BF16)
    _Stream(_held(_sweep(wq, 12, 0), W_LAG)).rest()

    @pl.loop(0, 2)
    def _(p):
        pair_stream(k_hbm, 0, p, maybe_first=True).rest()

    for mat in (wq, wo, w1):
        _wait_all(*mat[1:])
    att_s[...] = jnp.zeros(att_s.shape, F32)
    row = lax.broadcasted_iota(jnp.int32, (8, PAIR), 0)
    col = lax.broadcasted_iota(jnp.int32, (8, PAIR), 1)
    own = jnp.logical_or(jnp.logical_and(row == 0, col < DH), jnp.logical_and(row == 1, col >= DH))

    def scores(p, stream):
        slot = p % NSLOT
        step = len(stream.seq) // (ncol + 2)
        _wait_all(ring.at[slot], sem_kv.at[slot])
        q = jnp.where(own, _dot(h, wq_v[:, pl.ds(_aligned(p * PAIR, LANE), PAIR)]), 0.0).astype(BF16)
        stream.more(step)
        s = []
        for c in range(ncol):
            s.append(_dot(q, ring[slot, :, c * WIDE:(c + 1) * WIDE]) * DH ** -0.5)
            stream.more(step)
        s = jnp.concatenate(s, axis=1)
        e = jnp.exp(s - jnp.max(s, axis=-1, keepdims=True))
        p_s[p] = e / jnp.sum(e, axis=-1, keepdims=True)
        stream.rest()

    @pl.loop(0, NPAIR - 2)
    def _(p):
        scores(p, pair_stream(k_hbm, 0, p + 2))

    _Stream(_held(pair(k_hbm, 0, NPAIR - 1), KV_LAG)).rest()

    @pl.loop(NPAIR - 2, NPAIR)
    def _(p):
        scores(p, pair_stream(v_hbm, NPAIR, p + 2 - NPAIR, maybe_first=True))

    def weigh(p, c):
        cols = pl.ds(c * WIDE, WIDE)
        return lax.dot_general(p_s[p, :, cols].astype(BF16), ring[(NPAIR + p) % NSLOT, :, cols],
                               (((1,), (1,)), ((), ())), preferred_element_type=F32)

    def project(p, o):
        return _dot(jnp.where(own, o, 0.0).astype(BF16), wo_v[pl.ds(_aligned(p * PAIR, LANE), PAIR), :])

    def values(p, stream, step):
        slot = (NPAIR + p) % NSLOT
        _wait_all(ring.at[slot], sem_kv.at[slot])
        o = jnp.zeros((8, PAIR), F32)
        for c in range(ncol):
            o += weigh(p, c)
            stream.more(step)
        att_s[...] += project(p, o)

    @pl.loop(0, NPAIR - 3)
    def _(p):
        stream = pair_stream(v_hbm, NPAIR, p + 2)
        values(p, stream, len(stream.seq) // (ncol + 2))
        stream.rest()

    last = NPAIR - 1
    w2_parts = W2_MXU + tuple((rows,) for rows in W2_VPU)
    w2_seq = _queued([[functools.partial(_copy, w2_hbm, w2_v, sem_w2.at[i], pl.ds(r0 + r, SUB))]
                      for i, part in enumerate(w2_parts)
                      for r in range(0, max(n for _, n in part), SUB) for r0, n in part if r < n])
    seq = pair(v_hbm, NPAIR, last, PAIR // SUB, sem_last)
    held = _held(seq, KV_LAG)
    stream = _Stream(_lagged(seq, KV_LAG, _held(pair(v_hbm, NPAIR, last - 1), KV_LAG)) + held[:-W2_LAG]
                     + _lagged(w2_seq, W2_LAG, held[-W2_LAG:]) + _held(w2_seq, W2_LAG))
    values(last - 2, stream, len(seq) // (3 * ncol))
    stream.upto(len(seq) // 2)
    values(last - 1, stream, V_PACE)
    o = jnp.zeros((8, PAIR), F32)
    for i, c in enumerate(KV_COLS):
        stream.more(V_PACE)
        stream.upto((i + 1) * len(seq) // ncol + (V_LOOK if i < ncol - 1 else MLP_LOOK))
        _wait_all(ring.at[(NPAIR + last) % NSLOT, :, pl.ds(c * WIDE, WIDE)], sem_last.at[c])
        o += weigh(last, c)
    stream.more(MLP_PACE)
    att = att_s[...] + project(last, o)
    stream.more(MLP_PACE)

    x1 = x0 + mod(2) * jnp.broadcast_to(jnp.sum(att, axis=0, keepdims=True), (8, D))
    h2 = (_layernorm(x1) * (1.0 + mod(4)) + mod(3)).astype(BF16)
    stream.more(MLP_PACE)
    b1 = b1_v[...].astype(F32)
    act = []
    for i in range(F // WIDE):
        bias = jnp.concatenate(
            [jnp.broadcast_to(b1[t:t + 1, :], (8, LANE)) for t in range(i * PIECE, (i + 1) * PIECE)], axis=1)
        act.append(_mish(_dot(h2, w1_v[:, i * WIDE:(i + 1) * WIDE]) + bias).astype(BF16))
        stream.more(MLP_PACE)
    stream.rest()
    act = jnp.concatenate(act, axis=1)
    r_vpu = W2_VPU[0][0]
    act_s[...] = jnp.broadcast_to(act[0:1, r_vpu:].astype(F32), (LANE, F - r_vpu)).T
    y = jnp.zeros((8, D), F32)
    for i, part in enumerate(W2_MXU):
        for r0, n in part:
            _wait_all(w2_v.at[pl.ds(r0, n)], sem_w2.at[i])
        for r0, n in part:
            y += _dot(act[:, r0:r0 + n], w2_v[r0:r0 + n, :])
    y = jnp.where(lax.broadcasted_iota(jnp.int32, (8, D), 0) == 0, y, 0.0)
    for i, (r0, n) in enumerate(W2_VPU):
        _wait_all(w2_v.at[pl.ds(r0, n)], sem_w2.at[len(W2_MXU) + i])
        for r in range(r0, r0 + n, 2 * SUB):
            a = act_s[r - r_vpu:r - r_vpu + 2 * SUB, :]
            t = jnp.concatenate([a] * (D // LANE), axis=1) * w2_v[r:r + 2 * SUB, :].astype(F32)
            y = y + t[:SUB] + t[SUB:]
    y = jnp.sum(y, axis=0, keepdims=True)
    o_ref[...] = (x1[0:1] + mod(5)[0:1] * y).astype(o_ref.dtype)


@jax.jit
def pallas_adaLN_cond__sliding_block_cached__dense_activation_mish__decode_kernel(
    A_x: jax.Array,
    A_k_cache: jax.Array,
    A_v_cache: jax.Array,
    A_wq: jax.Array,
    A_wo: jax.Array,
    B_x: jax.Array,
    B_w1: jax.Array,
    B_b1: jax.Array,
    B_w2: jax.Array,
    c: jax.Array,
    w_mod: jax.Array,
):
    del B_x
    sk = A_k_cache.shape[2]
    window = min(4096, max(256, sk // 4))
    kt = jnp.swapaxes(A_k_cache, 2, 3).reshape(H * DH, sk)
    vt = jnp.swapaxes(A_v_cache, 2, 3).reshape(H * DH, sk)
    hbm = pl.BlockSpec(memory_space=pltpu.HBM)
    out = pl.pallas_call(
        _kernel,
        out_shape=jax.ShapeDtypeStruct((1, D), A_x.dtype),
        in_specs=[hbm] * 10,
        out_specs=pl.BlockSpec(memory_space=pltpu.VMEM),
        scratch_shapes=[
            pltpu.VMEM((1, D), BF16),
            pltpu.VMEM((1, D), BF16),
            pltpu.VMEM((F // LANE, LANE), BF16),
            pltpu.VMEM((D, 6 * D), BF16),
            pltpu.VMEM((D, H * DH), BF16),
            pltpu.VMEM((H * DH, D), BF16),
            pltpu.VMEM((D, F), BF16),
            pltpu.VMEM((F, D), BF16),
            pltpu.VMEM((NSLOT, PAIR, window), BF16),
            pltpu.VMEM((NPAIR, 8, window), F32),
            pltpu.VMEM((8, D), F32),
            pltpu.VMEM((8, 6 * D), F32),
            pltpu.VMEM((F - W2_VPU[0][0], LANE), F32),
            pltpu.SemaphoreType.DMA((7,)),
            pltpu.SemaphoreType.DMA((NSLOT,)),
            pltpu.SemaphoreType.DMA((len(KV_COLS),)),
            pltpu.SemaphoreType.DMA((len(W2_MXU) + len(W2_VPU),)),
        ],
        compiler_params=pltpu.CompilerParams(
            vmem_limit_bytes=64 * 2**20,
            disable_bounds_checks=True,
            disable_semaphore_checks=True,
        ),
        name="adaln_attn_mlp_decode",
    )(A_x.reshape(1, D), kt, vt, A_wq, A_wo, B_w1, B_b1.reshape(F // LANE, LANE), B_w2, c, w_mod)
    return out.reshape(A_x.shape)
```

```python
import functools

import jax
import jax.numpy as jnp
from jax import lax
import jax.experimental.pallas as pl
import jax.experimental.pallas.tpu as pltpu

D = 640
H = 32
DH = 192
F = 1536
PAIR = 2 * DH
NPAIR = H // 2
LANE = 128
SUB = 8
PIECE = 4
WIDE = PIECE * LANE
STRIPE = 64
F32 = jnp.float32
BF16 = jnp.bfloat16

NSLOT = 3
KV_COLS = (5, 6, 7, 4, 3, 0, 1, 2)
KV_CYCLE = ((0, 1), (1, 2), (1, 3))
W_CYCLE = (0, 1, 1, 1, 1, 1)
KV_LAG, W_LAG, W2_LAG = 13, 4, 4
W2_MXU = (((0, 256), (384, 256), (768, 256), (1152, 128)), ((256, 128), (640, 128), (1024, 128)))
W2_VPU = ((1280, 128), (1408, 64), (1472, 48), (1520, 16))
V_PACE, V_LOOK = 8, 64
MLP_PACE, MLP_LOOK = 20, 96


def _layernorm(x, eps=1e-5):
    m = jnp.mean(x, axis=-1, keepdims=True)
    d = x - m
    v = jnp.mean(d * d, axis=-1, keepdims=True)
    return d / jnp.sqrt(v + eps)


def _mish(u):
    softplus = jnp.log1p(jnp.exp(-jnp.abs(u))) + jnp.where(u > 0, u, 0.0)
    return u * jnp.tanh(softplus)


def _dot(a, b):
    return jnp.dot(a, b, preferred_element_type=F32)


def _aligned(i, n):
    return i if isinstance(i, int) else pl.multiple_of(i, n)


def _copy(src, dst, sem, idx, queue):
    pltpu.make_async_copy(src.at[idx], dst.at[idx], sem).start(priority=queue)


def _wait_all(buf, sem):
    pltpu.make_async_copy(buf, buf, sem).wait()


def _piece(src, dst, sem, i):
    width = src.shape[1] // LANE
    starts, t, end = [], i * PIECE, (i + 1) * PIECE
    while t < end:
        r, c = divmod(t, width)
        n = min(end - t, width - c)
        starts.append(functools.partial(_copy, src, dst, sem, (pl.ds(r * SUB, SUB), pl.ds(c * LANE, n * LANE))))
        t += n
    return starts


def _queued(pieces):
    return [(W_CYCLE[i % len(W_CYCLE)], starts) for i, starts in enumerate(pieces)]


def _walk(mats, cols):
    return _queued([_piece(*m, i) for c in cols for m in mats
                    for i in range(c, m[0].size // (SUB * WIDE), STRIPE)])


def _sweep(mat, period, i):
    src, dst, sem = mat
    rows = period * WIDE // src.shape[1] * SUB
    view = pl.ds(_aligned(i * rows, SUB), src.shape[0] - (STRIPE // period - 1) * rows)
    return _queued([_piece(src.at[view], dst.at[view], sem, r + c) for c in reversed(range(period))
                    for r in range(0, src.size // (SUB * WIDE), STRIPE)])


def _held(seq, lag):
    zero = [x for x in seq if x[0] == 0]
    return zero[len(zero) - lag:]


def _lagged(seq, lag, held=(), valid=None):
    if valid is not None:
        held = [(0, [lambda q, s=s: pl.when(valid)(lambda: s(q)) for s in starts]) for _, starts in held]
    zero = [x for x in seq if x[0] == 0]
    zero = iter([None] * (lag - len(held)) + list(held) + zero[:len(zero) - lag])
    return [x for x in (next(zero) if x[0] == 0 else x for x in seq) if x is not None]


class _Stream:
    def __init__(self, seq):
        self.seq = seq
        self.pos = 0

    def upto(self, n):
        while self.pos < min(n, len(self.seq)):
            queue, starts = self.seq[self.pos]
            for start in starts:
                start(queue)
            self.pos += 1

    def more(self, n):
        self.upto(self.pos + n)

    def rest(self):
        self.upto(len(self.seq))


def _kernel(x_hbm, k_hbm, v_hbm, wq_hbm, wo_hbm, w1_hbm, b1_hbm, w2_hbm, c_hbm, wmod_hbm, o_ref,
            x_v, c_v, b1_v, wmod_v, wq_v, wo_v, w1_v, w2_v, ring, p_s, att_s, mod_s, act_s,
            sem_w, sem_kv, sem_last, sem_w2):
    window = ring.shape[2]
    ncol = len(KV_COLS)
    assert window == ncol * WIDE
    small = [pltpu.make_async_copy(s, d, sem_w.at[i])
             for i, (s, d) in enumerate(((c_hbm, c_v), (x_hbm, x_v), (b1_hbm, b1_v)))]
    wmod, wq, wo, w1 = [(s, d, sem_w.at[len(small) + i]) for i, (s, d) in enumerate(
        ((wmod_hbm, wmod_v), (wq_hbm, wq_v), (wo_hbm, wo_v), (w1_hbm, w1_v)))]

    def pair(src, base, p, run=DH // SUB, sems=None):
        slot = (base + p) % NSLOT
        src = src.at[pl.ds(_aligned(p * PAIR, LANE), PAIR), pl.ds(src.shape[1] - window, window)]
        dst, sem = ring.at[slot], sem_kv.at[slot]
        seq = []
        for r0 in range(0, PAIR // SUB, run):
            for c in KV_COLS:
                r = r0
                while r < r0 + run:
                    queue, n = KV_CYCLE[len(seq) % len(KV_CYCLE)]
                    idx = (pl.ds(r * SUB, n * SUB), pl.ds(c * WIDE, WIDE))
                    seq.append((queue, [functools.partial(
                        _copy, src, dst, sem if sems is None else sems.at[c], idx)]))
                    r += n
                assert r == r0 + run
        return seq

    def pair_stream(src, base, p, maybe_first=False):
        held = _held(pair(src, base, jnp.maximum(p - 1, 0)), KV_LAG)
        return _Stream(_lagged(pair(src, base, p), KV_LAG, held, p > 0 if maybe_first else None))

    def sweep_stream(mat, period, i):
        last = STRIPE // period - 1
        held = _held(_sweep(mat, period, jnp.minimum(last - i + 1, last)), W_LAG)
        return _Stream(_lagged(_sweep(mat, period, last - i), W_LAG, held, i > 0))

    odd_cols = range(STRIPE - 1, 59, -1)
    seq = _walk((wmod, w1), range(STRIPE - 1, -1, -1)) + _walk((wo,), odd_cols)
    stream = _Stream(_lagged(seq, W_LAG) + _held(seq, W_LAG))
    stream.more(len(W_CYCLE))
    for cp in small:
        cp.start()
    stream.rest()

    @pl.loop(0, 12)
    def _(i):
        sweep_stream(wo, 5, i).rest()

    seq = _walk((wq,), odd_cols)
    _Stream(_lagged(seq, W_LAG, _held(_sweep(wo, 5, 0), W_LAG)) + _held(seq, W_LAG)).rest()
    for cp in small:
        cp.wait()
    _wait_all(*wmod[1:])
    cf = c_v[...].astype(F32)
    silu_c = jnp.broadcast_to(cf * jax.nn.sigmoid(cf), (8, D)).astype(BF16)

    @pl.loop(0, 5)
    def _(i):
        stream = sweep_stream(wq, 12, i)
        n = 6 * D // 10
        for j in range(2):
            stream.more(len(stream.seq) // 3)
            cols = pl.ds(_aligned((2 * i + j) * n, LANE), n)
            mod_s[:, cols] = _dot(silu_c, wmod_v[:, cols])
        stream.rest()

    def mod(i):
        return mod_s[:, i * D:(i + 1) * D]

    x0 = jnp.broadcast_to(x_v[...].astype(F32), (8, D))
    h = (_layernorm(x0) * (1.0 + mod(1)) + mod(0)).astype(BF16)
    _Stream(_held(_sweep(wq, 12, 0), W_LAG)).rest()

    @pl.loop(0, 2)
    def _(p):
        pair_stream(k_hbm, 0, p, maybe_first=True).rest()

    for mat in (wq, wo, w1):
        _wait_all(*mat[1:])
    att_s[...] = jnp.zeros(att_s.shape, F32)
    row = lax.broadcasted_iota(jnp.int32, (8, PAIR), 0)
    col = lax.broadcasted_iota(jnp.int32, (8, PAIR), 1)
    own = jnp.logical_or(jnp.logical_and(row == 0, col < DH), jnp.logical_and(row == 1, col >= DH))

    def scores(p, stream):
        slot = p % NSLOT
        step = len(stream.seq) // (ncol + 2)
        _wait_all(ring.at[slot], sem_kv.at[slot])
        q = jnp.where(own, _dot(h, wq_v[:, pl.ds(_aligned(p * PAIR, LANE), PAIR)]), 0.0).astype(BF16)
        stream.more(step)
        s = []
        for c in range(ncol):
            s.append(_dot(q, ring[slot, :, c * WIDE:(c + 1) * WIDE]) * DH ** -0.5)
            stream.more(step)
        s = jnp.concatenate(s, axis=1)
        e = jnp.exp(s - jnp.max(s, axis=-1, keepdims=True))
        p_s[p] = e / jnp.sum(e, axis=-1, keepdims=True)
        stream.rest()

    @pl.loop(0, NPAIR - 2)
    def _(p):
        scores(p, pair_stream(k_hbm, 0, p + 2))

    _Stream(_held(pair(k_hbm, 0, NPAIR - 1), KV_LAG)).rest()

    @pl.loop(NPAIR - 2, NPAIR)
    def _(p):
        scores(p, pair_stream(v_hbm, NPAIR, p + 2 - NPAIR, maybe_first=True))

    def weigh(p, c):
        cols = pl.ds(c * WIDE, WIDE)
        return lax.dot_general(p_s[p, :, cols].astype(BF16), ring[(NPAIR + p) % NSLOT, :, cols],
                               (((1,), (1,)), ((), ())), preferred_element_type=F32)

    def project(p, o):
        return _dot(jnp.where(own, o, 0.0).astype(BF16), wo_v[pl.ds(_aligned(p * PAIR, LANE), PAIR), :])

    def values(p, stream, step):
        slot = (NPAIR + p) % NSLOT
        _wait_all(ring.at[slot], sem_kv.at[slot])
        o = jnp.zeros((8, PAIR), F32)
        for c in range(ncol):
            o += weigh(p, c)
            stream.more(step)
        att_s[...] += project(p, o)

    @pl.loop(0, NPAIR - 3)
    def _(p):
        stream = pair_stream(v_hbm, NPAIR, p + 2)
        values(p, stream, len(stream.seq) // (ncol + 2))
        stream.rest()

    last = NPAIR - 1
    w2_parts = W2_MXU + tuple((rows,) for rows in W2_VPU)
    w2_seq = _queued([[functools.partial(_copy, w2_hbm, w2_v, sem_w2.at[i], pl.ds(r0 + r, SUB))]
                      for i, part in enumerate(w2_parts)
                      for r in range(0, max(n for _, n in part), SUB) for r0, n in part if r < n])
    seq = pair(v_hbm, NPAIR, last, PAIR // SUB, sem_last)
    held = _held(seq, KV_LAG)
    stream = _Stream(_lagged(seq, KV_LAG, _held(pair(v_hbm, NPAIR, last - 1), KV_LAG)) + held[:-W2_LAG]
                     + _lagged(w2_seq, W2_LAG, held[-W2_LAG:]) + _held(w2_seq, W2_LAG))
    values(last - 2, stream, len(seq) // (3 * ncol))
    stream.upto(len(seq) // 2)
    values(last - 1, stream, V_PACE)
    o = jnp.zeros((8, PAIR), F32)
    assert KV_LAG * len(KV_CYCLE) <= V_LOOK
    for i, c in enumerate(KV_COLS):
        stream.more(V_PACE)
        stream.upto((i + 1) * len(seq) // ncol + (V_LOOK if i < ncol - 1 else MLP_LOOK))
        _wait_all(ring.at[(NPAIR + last) % NSLOT, :, pl.ds(c * WIDE, WIDE)], sem_last.at[c])
        o += weigh(last, c)
    stream.more(MLP_PACE)
    att = att_s[...] + project(last, o)
    stream.more(MLP_PACE)

    x1 = x0 + mod(2) * jnp.broadcast_to(jnp.sum(att, axis=0, keepdims=True), (8, D))
    h2 = (_layernorm(x1) * (1.0 + mod(4)) + mod(3)).astype(BF16)
    stream.more(MLP_PACE)
    b1 = b1_v[...].astype(F32)
    act = []
    for i in range(F // WIDE):
        bias = jnp.concatenate(
            [jnp.broadcast_to(b1[t:t + 1, :], (8, LANE)) for t in range(i * PIECE, (i + 1) * PIECE)], axis=1)
        act.append(_mish(_dot(h2, w1_v[:, i * WIDE:(i + 1) * WIDE]) + bias).astype(BF16))
        stream.more(MLP_PACE)
    stream.rest()
    act = jnp.concatenate(act, axis=1)
    r_vpu = W2_VPU[0][0]
    act_s[...] = jnp.broadcast_to(act[0:1, r_vpu:].astype(F32), (LANE, F - r_vpu)).T
    y = jnp.zeros((8, D), F32)
    for i, part in enumerate(W2_MXU):
        for r0, n in part:
            _wait_all(w2_v.at[pl.ds(r0, n)], sem_w2.at[i])
        for r0, n in part:
            y += _dot(act[:, r0:r0 + n], w2_v[r0:r0 + n, :])
    y = jnp.where(lax.broadcasted_iota(jnp.int32, (8, D), 0) == 0, y, 0.0)
    for i, (r0, n) in enumerate(W2_VPU):
        _wait_all(w2_v.at[pl.ds(r0, n)], sem_w2.at[len(W2_MXU) + i])
        for r in range(r0, r0 + n, 2 * SUB):
            a = act_s[r - r_vpu:r - r_vpu + 2 * SUB, :]
            t = jnp.concatenate([a] * (D // LANE), axis=1) * w2_v[r:r + 2 * SUB, :].astype(F32)
            y = y + t[:SUB] + t[SUB:]
    y = jnp.sum(y, axis=0, keepdims=True)
    o_ref[...] = (x1[0:1] + mod(5)[0:1] * y).astype(o_ref.dtype)


@jax.jit
def pallas_adaLN_cond__sliding_block_cached__dense_activation_mish__decode_kernel(
    A_x: jax.Array,
    A_k_cache: jax.Array,
    A_v_cache: jax.Array,
    A_wq: jax.Array,
    A_wo: jax.Array,
    B_x: jax.Array,
    B_w1: jax.Array,
    B_b1: jax.Array,
    B_w2: jax.Array,
    c: jax.Array,
    w_mod: jax.Array,
):
    del B_x
    sk = A_k_cache.shape[2]
    window = min(4096, max(256, sk // 4))
    kt = jnp.swapaxes(A_k_cache, 2, 3).reshape(H * DH, sk)
    vt = jnp.swapaxes(A_v_cache, 2, 3).reshape(H * DH, sk)
    hbm = pl.BlockSpec(memory_space=pltpu.HBM)
    out = pl.pallas_call(
        _kernel,
        out_shape=jax.ShapeDtypeStruct((1, D), A_x.dtype),
        in_specs=[hbm] * 10,
        out_specs=pl.BlockSpec(memory_space=pltpu.VMEM),
        scratch_shapes=[
            pltpu.VMEM((1, D), BF16),
            pltpu.VMEM((1, D), BF16),
            pltpu.VMEM((F // LANE, LANE), BF16),
            pltpu.VMEM((D, 6 * D), BF16),
            pltpu.VMEM((D, H * DH), BF16),
            pltpu.VMEM((H * DH, D), BF16),
            pltpu.VMEM((D, F), BF16),
            pltpu.VMEM((F, D), BF16),
            pltpu.VMEM((NSLOT, PAIR, window), BF16),
            pltpu.VMEM((NPAIR, 8, window), F32),
            pltpu.VMEM((8, D), F32),
            pltpu.VMEM((8, 6 * D), F32),
            pltpu.VMEM((F - W2_VPU[0][0], LANE), F32),
            pltpu.SemaphoreType.DMA((7,)),
            pltpu.SemaphoreType.DMA((NSLOT,)),
            pltpu.SemaphoreType.DMA((len(KV_COLS),)),
            pltpu.SemaphoreType.DMA((len(W2_MXU) + len(W2_VPU),)),
        ],
        compiler_params=pltpu.CompilerParams(
            vmem_limit_bytes=64 * 2**20,
            disable_bounds_checks=True,
            disable_semaphore_checks=True,
        ),
        name="adaln_attn_mlp_decode",
    )(A_x.reshape(1, D), kt, vt, A_wq, A_wo, B_w1, B_b1.reshape(F // LANE, LANE), B_w2, c, w_mod)
    return out.reshape(A_x.shape)
```
